```python
import os as _os
_os.environ.setdefault("JAX_PLATFORMS", "cpu")
import jax
import jax.numpy as jnp

def _softmax(x, axis=-1):
    return jax.nn.softmax(x, axis=axis)
def _gelu(x):
    return jax.nn.gelu(x, approximate=True)
def _silu(x):
    return jax.nn.silu(x)
def _sigmoid(x):
    return jax.nn.sigmoid(x)
def _layernorm(x, axis=-1, eps=1e-5):
    m = jnp.mean(x, axis=axis, keepdims=True)
    v = jnp.var(x, axis=axis, keepdims=True)
    return (x - m) / jnp.sqrt(v + eps)
def _scatter_add(tgt, idx, src, axis=0):
    return tgt.at[idx].add(src)
def _segment_sum(src, seg, n):
    return jax.ops.segment_sum(src, seg, n)
class _Rng:
    def __init__(self, key):
        self._k = key
    def _next(self):
        self._k, sub = jax.random.split(self._k)
        return sub
    def normal(self, shape):
        return jax.random.normal(self._next(), shape, dtype=jnp.bfloat16)
    def randint(self, lo, hi, shape):
        return jax.random.randint(self._next(), shape, lo, hi, dtype=jnp.int32)
    def uniform(self, shape, lo=0.0, hi=1.0):
        return jax.random.uniform(self._next(), shape, jnp.bfloat16, lo, hi)
    def permutation(self, n):
        return jax.random.permutation(self._next(), n)


kernel_name = 'interleave_layers__linear_kernel_hedgehog__sliding_block__prompt'

def setup_inputs():
    _rng = _Rng(jax.random.key(int.from_bytes(__import__("os").urandom(4), "little")))
    _w = (lambda a: (lambda t: t.astype(jnp.bfloat16) if jnp.issubdtype(t.dtype, jnp.floating) else t)(jnp.asarray(a)))
    def _A_setup():
        B, S, D, H = 1, 2048, 448, 16
        Dh = D // H
        return {
            "x": _w((lambda *s: _rng.normal(s) * 0.05)(B, S, D)),
            "wqkv": _w((lambda *s: _rng.normal(s) * 0.4)(D, 3 * D)),
            "w_phi": _w((lambda *s: _rng.normal(s) * 0.4)(H, Dh, Dh) * (Dh ** -0.5)),
            "wo": _w((lambda *s: _rng.normal(s) * 0.05)(D, D)),
        }
    _A_in = _A_setup()

    def _B_setup():
        B, S, D = 1, 2048, 448
        return {
            "x": _w((lambda *s: _rng.normal(s) * 0.05)(B, S, D)),
            "wqkv": _w((lambda *s: _rng.normal(s) * 0.1)(D, 3 * D)),
            "wo": _w((lambda *s: _rng.normal(s) * 0.1)(D, D)),
        }
    _B_in = _B_setup()

    return {
        "A_x": _A_in["x"],
        "A_wqkv": _A_in["wqkv"],
        "A_w_phi": _A_in["w_phi"],
        "A_wo": _A_in["wo"],
        "B_x": _B_in["x"],
        "B_wqkv": _B_in["wqkv"],
        "B_wo": _B_in["wo"],
    }

def reference(A_x, A_wqkv, A_w_phi, A_wo, B_x, B_wqkv, B_wo):
    def _A_ref(x, wqkv, w_phi, wo):
        B, S, D = x.shape
        H = 16; Dh = D // H
        qkv = (lambda x, *d: x.transpose(*d))((x @ wqkv).reshape(B, S, 3, H, Dh), 2, 0, 3, 1, 4)
        q, k, v = qkv[0], qkv[1], qkv[2]
        pq = jnp.einsum("bhsd,hdf->bhsf", q, w_phi)
        pk = jnp.einsum("bhsd,hdf->bhsf", k, w_phi)
        phi_q = jnp.concatenate([_softmax(pq, axis=-1), _softmax(-pq, axis=-1)], axis=-1)
        phi_k = jnp.concatenate([_softmax(pk, axis=-1), _softmax(-pk, axis=-1)], axis=-1)
        kv = jnp.einsum("bhsf,bhsd->bhfd", phi_k, v)
        z  = jnp.einsum("bhsf->bhf", phi_k)
        num = jnp.einsum("bhqf,bhfd->bhqd", phi_q, kv)
        den = jnp.einsum("bhqf,bhf->bhq", phi_q, z)[..., None] + 1e-6
        o = num / den
        return (lambda x, *d: x.transpose(*d))(o, 0, 2, 1, 3).reshape(B, S, D) @ wo

    def _B_ref(x, wqkv, wo):
        B, S, D = x.shape
        H = 16; Dh = D // H; W = 256
        qkv = (lambda x, *d: x.transpose(*d))((x @ wqkv).reshape(B, S, 3, H, Dh), 2, 0, 3, 1, 4)
        q, k, v = qkv[0], qkv[1], qkv[2]
        scores = jnp.einsum("bhqd,bhkd->bhqk", q, k) * (Dh ** -0.5)
        idx = jnp.arange(S)
        mask = (idx[:, None] - idx[None, :] >= 0) & (idx[:, None] - idx[None, :] < W)
        scores = jnp.where(mask[None, None], scores, -1e9)
        p = _softmax(scores, axis=-1)
        o = jnp.einsum("bhqk,bhkd->bhqd", p, v)
        return (lambda x, *d: x.transpose(*d))(o, 0, 2, 1, 3).reshape(B, S, D) @ wo

    x = A_x
    x = x + _A_ref(_layernorm(x, axis=-1), A_wqkv, A_w_phi, A_wo)
    x = x + _B_ref(_layernorm(x, axis=-1), B_wqkv, B_wo)
    x = x + _A_ref(_layernorm(x, axis=-1), A_wqkv, A_w_phi, A_wo)
    x = x + _B_ref(_layernorm(x, axis=-1), B_wqkv, B_wo)
    return x
```

```python
import functools

import numpy as np
import jax
import jax.numpy as jnp
from jax import lax
import jax.experimental.pallas as pl
import jax.experimental.pallas.tpu as pltpu

S, D, H, DH = 2048, 448, 16, 28
NP, NG = H // 2, H // 4
T = 128
NTILE = S // T
NPAIR = NTILE // 2
HALF = D // 2
EARLY = 6
LOG2E = float(np.log2(np.e))
NEG = -1e30
F32, BF16, U32 = jnp.float32, jnp.bfloat16, jnp.uint32
AQ, AK, AV, AO, BQ, BK, BV, BO = range(8)
NN = (((1,), (0,)), ((), ()))
NT = (((1,), (1,)), ((), ()))
ORDER0 = "KKKKkkKkKkQKQkkKkKkkkqqQkkqkkqnnkqqQnQqQqQqKnqqqmqKkKqqmqKmKKmKKK"
ORDER1 = "AAAbccccxSSOAOOObssxssSOOsObSsobAosAsAsssossssxSSAAoPAAKaasKPkksxSKsSaKssakssKFsskkskFPFsKxKksFFSkksQQkkksQFsSskkssQkFqskxqsQqssPQsSFsKssQKqFqsFFSqKPxssssqqFqsKsSqPKqKqKSxKqssFsSsFsFsqsFqsqssssPFFSKsKsFFssPFK"
ORDER2 = "AbccxSAbAccOsASObsbAAssssssxPSASAAOOsAsssssssPAaxSOSaaassFsFOsssssxFPSFFSsFFFsxssFssxssPFSsOssSsSsxsssFsssSsPFSsFSsxssPsssFsssFSFsFsssPFssSssssFFFP"
BRIDGE1 = "RccccOOOORORROORooRtooKRKKKkkkKkkkktkKQKKkKkkQKkQkQKKKkkKKQkKKKzAAEAAbbEEQbbAAAAAqEAqqAdQdddaqEEaaEaEqEFFFEEqFqFeeeFtqFtFtqFFtFtFqeqtFqFqtFFqttFFtqtFqtFttF"
FIRST = "FFxSSFxFsssssSsssPsxsFssFSFsssSsSxPssssSxssSFssPssssFSSFsFxsssPsSsssxssFssPsSsssFSssxssFsFsPssSSFsFFsssPssSFssFFssssP"
LAST1 = "ccccOxOSxsSssOSxssssOsPSssssOSOxsssSsPOosoosssssssSosxSKsssPKksksKKksKskkkKkkKPkkKkkkSxkKSskkssSxKKsssssPsSSsSssxKsssssssPsKssSssPKssSKssKsKssKsP"
LAST2 = "ccccOxxSOOssSssssOsxSsPsSssOSsOsssssxsPssSSsSsssPssOsxsSxSSsssSssxsSssPSssxsSsssPssSssssPsssssssssPsssssssP"
START = "wKwKwKwKwKwkKkKkkKkkKkkKkkKkkKkkKkkKKKKKwnnwnnwnnwnnwmmmm"
BRIDGE0 = "wKKwwwwwQwRKwRwwKwQRwwKwwQwwwwKwRKwwKwKwwRwKwwQwKkkRkkKkqKkKtRtQkkKqtQtttQkKkkkKkkkkKqqqqttqqttttttttqqqqqzqAqAAAbbEEbEbAAAAAAEAqaaaaddFdFdFFFFFFFFEEEEFFFEFFEFFFEFeeFeFe"


def _dot(a, b, dn=NN):
    return lax.dot_general(a, b, dn, preferred_element_type=F32)


def _iota(shape, dim):
    return lax.broadcasted_iota(jnp.int32, shape, dim)


def _load(ref, *index):
    return ref.bitcast(U32)[index]


def _bf16(x):
    return pltpu.bitcast(x, BF16)


def _cat(xs, axis=0):
    return jnp.concatenate(xs, axis=axis)


def _recip(x):
    r = pl.reciprocal(x, approx=True)
    return r * (2.0 - x * r)


def _tree(xs, op):
    while len(xs) > 1:
        xs = [op(xs[i], xs[i + 1]) if i + 1 < len(xs) else xs[i] for i in range(0, len(xs), 2)]
    return xs[0]


def _slabs(x):
    return [x[i:i + 8] for i in range(0, x.shape[0], 8)]


def _allreduce(xs, op, shifts):
    r = _tree(xs, op)
    for s in shifts:
        r = op(r, pltpu.roll(r, s, 0))
    return r


def _moments(x):
    xs = _slabs(x)
    mean = _tree(xs, jnp.add) * (1.0 / len(xs))
    return mean, _tree([(v - mean) * (v - mean) for v in xs], jnp.add)


def _operands(dst, load):
    for n in range(0, HALF // 8, 2):
        ops = []
        for c in (n, n + 1):
            b11, b12, b21, b22 = load(0, c), load(1, c), load(0, c + HALF // 8), load(1, c + HALF // 8)
            ops.append((b11 + b22, b11, b12 - b22, b21 - b11, b22, b11 + b12, b21 + b22))
        for m in range(7):
            dst(m, pl.ds(8 * n, 16), _cat([ops[0][m], ops[1][m]]).astype(BF16))
        if n in (4, 12, 18, 26):
            yield


def _statistics(parts):
    assert len(parts) == NG
    mean = _allreduce([m for m, _ in parts], jnp.add, (4, 2, 1)) * (1.0 / (8 * NG))
    sq = [s + (D / (8 * NG)) * ((m - mean) * (m - mean)) for m, s in parts]
    return mean, lax.rsqrt(_allreduce(sq, jnp.add, (4, 2, 1)) * (1.0 / D) + 1e-5)


def _layernorm(statistics, load, dst):
    stats = [statistics(t) for t in range(2)]
    yield from _operands(dst, lambda t, n: (load(t, n) - stats[t][0]) * stats[t][1])


def _feature_map(p):
    xs = _slabs(p)
    hi = _allreduce(xs, jnp.maximum, (4, 2))
    lo = _allreduce(xs, jnp.minimum, (4, 2))
    ep = [jnp.exp2(v - hi) for v in xs]
    en = [jnp.exp2(lo - v) for v in xs]
    rp = _recip(_allreduce(ep, jnp.add, (4, 2)))
    rn = _recip(_allreduce(en, jnp.add, (4, 2)))
    return _cat([e * rp for e in ep] + [e * rn for e in en]).astype(BF16)


def _kernel(x_hbm, wa_hbm, wphi_hbm, woa_hbm, wb_hbm, wob_hbm, o_hbm,
            xin, wa_in, wphi, woa_in, wb_in, wob_in, ost,
            wt, ws, xs, lna, phiq, kv, kvb, lnb, att, qf, kf, kprev, kx, vext, pre, phik, lin, lat, sbuf, stats, pst,
            zero_ref, isem, osem):
    def window(src, dst, lo, hi):
        return src.at[:, pl.ds(lo, hi - lo)], dst.at[:, pl.ds(lo, hi - lo)]

    copies = [pltpu.make_async_copy(src, dst, isem.at[n]) for n, (src, dst) in enumerate([
        (wphi_hbm, wphi), window(x_hbm, xin, 0, 2 * T), window(wa_hbm, wa_in, 384, 896),
        window(wa_hbm, wa_in, 896, 3 * D), window(wa_hbm, wa_in, 0, 384), window(x_hbm, xin, 2 * T, 6 * T),
        window(x_hbm, xin, 6 * T, S), (woa_hbm, woa_in), (wb_hbm, wb_in), (wob_hbm, wob_in)])]
    for cp in copies[:EARLY]:
        cp.start()

    zero_ref[0] = 0

    def cols(i, n):
        return pl.ds(i * n if isinstance(i, int) else pl.multiple_of(i * n, n), n)

    def out_copy(j):
        return pltpu.make_async_copy(ost.at[j], o_hbm.at[:, cols(j, 2 * T)], osem.at[j])

    def transpose_weight(src, lo, hi):
        for c in range(lo, hi, 128):
            w = min(128, hi - c)
            for j, (k0, k1) in enumerate(((0, 128), (128, HALF), (HALF, HALF + 128), (HALF + 128, D))):
                blk = src[k0:k1, c:c + w].astype(F32)
                if k1 - k0 < 128:
                    blk = _cat([blk, jnp.zeros((128 - k1 + k0, w), F32)])
                wt[j, c:c + w, :] = blk.T
            yield

    def weight_operands(slot, part, fold=None):
        for g in range(2):
            halves = []
            for c in (g, g + 2):
                rows = _cat([wt[j, pl.ds(D * part + 112 * c, 112), :] for j in range(4)], axis=1)
                halves.append(rows if fold is None else _dot(fold[c], rows.astype(BF16)) * LOG2E)
            (a11, a12), (a21, a22) = [(half[:, :256], half[:, 256:]) for half in halves]
            for m, op in enumerate((a11 + a22, a21 + a22, a11, a22, a11 + a12, a21 - a11, a12 - a22)):
                for c in range(2):
                    ws[slot, m, g, c] = op[:, 128 * c:128 * c + 128].astype(BF16)
            yield

    r = _iota((112, D), 0)
    rh = (r >= 28).astype(jnp.int32) + (r >= 56).astype(jnp.int32) + (r >= 84).astype(jnp.int32)
    src_row = (r - 28 * rh) * H + rh
    r2 = _iota((112, DH), 0)
    pick = ((jnp.where(r2 >= 56, r2 - 56, r2) >> 1) == _iota((112, DH), 1)).astype(F32).astype(BF16)
    r3, c3 = _iota((112, 112), 0), _iota((112, 112), 1)
    lo3 = 28 * (jnp.where(r3 >= 56, 2, 0) + (r3 & 1))
    same = (c3 >= lo3) & (c3 < lo3 + 28)
    gather = [(_iota((112, D), 1) == src_row + 4 * g).astype(F32).astype(BF16) for g in range(NG)]
    copies[0].wait()
    copies[6].start()
    wg = [_dot(gather[g], wphi[...]).astype(BF16) for g in range(NG)]
    bd = [jnp.where(same, _dot(pick, wg[g], NT), 0.0).astype(BF16) for g in range(NG)]

    sub = _iota((8, T), 0)
    z = zero_ref[0]
    low = sub < 4
    lane = _iota((8, T), 1)

    def project(slot, at, finish):
        count, (rhs, at) = 0, at
        for g in range(2):
            m = {}
            for n in (0, 3, 4, 6, 2, 1, 5):
                b = _cat([_load(rhs, at, n + z), jnp.zeros((128 - HALF // 2, T), U32)])
                m[n] = _dot(_bf16(_cat([_load(ws, slot, n, g, c) for c in range(2)], axis=1)), _bf16(b))
                if n == 6:
                    finish(g, 0, m[0] + m[3] - m[4] + m[6])
                elif n == 2:
                    finish(g, 1, m[2] + m[4])
                elif n == 1:
                    finish(g + 2, 0, m[1] + m[3])
                elif n == 5:
                    finish(g + 2, 1, m[0] + m[2] - m[1] + m[5])
                count += 1
                if count % 2 == 0:
                    yield

    def into(ref, at):
        def store(m, rows, value):
            ref[at, m, rows, :] = value
        return store

    def stash(buf):
        def finish(g, t, y):
            buf[t, 112 * g:112 * g + 112, :] = y
        return finish

    def features(src, store):
        for g in (0, 2, 1, 3):
            for t in range(2):
                for p in (2 * g, 2 * g + 1):
                    store(t, p, _feature_map(src[t + z, 56 * p:56 * p + 56, :]))
                    yield

    def a_keys(j, first=False):
        vone = {}

        def values(g, t, v):
            for u in range(2):
                vone[2 * g + u, t] = _cat([jnp.ones((8, T), F32), v[56 * u:56 * u + 56]]).astype(BF16)

        def store(t, p, phi):
            phik[p, t] = phi

        def matmuls():
            yield from project(AK, (lna, j), stash(pre.at[0]))
            yield from project(AV, (lna, j), values)
            for p in (0, 1, 4, 5, 2, 3, 6, 7):
                upd = _dot(_cat([vone[p, 0], vone[p, 1]], axis=1), _bf16(_cat([_load(phik, p + z, t) for t in range(2)], axis=1)), NT)
                kv[p] = upd if first else kv[p] + upd
                if p % 2:
                    yield

        return dict(K=matmuls(), k=features(pre.at[0], store))

    def a_queries(j, names="Qq", slot=1):
        def store(t, p, phi):
            phiq[2 * j + t, p] = phi

        return dict(zip(names, (project(AQ, (lna, j), stash(pre.at[slot])), features(pre.at[slot], store))))

    def a_finalize():
        rr, cc = _iota((64, 112), 0), _iota((64, 112), 1)
        keep = (((rr >= 4) & (rr < 8)) | (rr >= 36)) == ((cc & 1) == 1)
        for p in range(NP):
            kvb[p] = jnp.where(keep, kv[p], 0.0).astype(BF16)
        yield

    def residual(j, moments):
        def finish(g, t, y):
            rows = pl.ds(112 * g, 112)
            x = y + xs[2 * j + t, rows, :]
            xs[2 * j + t, rows, :] = x
            moments[t].append(_moments(x))
        return finish

    def stream(j):
        return lambda t, n: xs[2 * j + t, 8 * n:8 * n + 8, :]

    def a_output(j, names="Aba", slot=0):
        moments, outs = ([], []), {}

        def matmuls():
            for p in (0, 4, 1, 5, 2, 6, 3, 7):
                for t in range(2):
                    nd = _dot(kvb[p], _bf16(_load(phiq, 2 * j + t, p)))
                    rc = _recip(nd[0:8] + 1e-6)
                    sw = pltpu.roll(rc, 4, 0)
                    ra, rb = jnp.where(low, rc, sw), jnp.where(low, sw, rc)
                    for n in range(7):
                        outs[t, 7 * p + n] = nd[8 * n + 8:8 * n + 16] * (ra if n < 3 else rc if n == 3 else rb)
                if p >= 4:
                    yield
            yield from project(AO, (lin, 0), residual(j, moments))

        return dict(zip(names, (matmuls(), _operands(into(lin, 0), lambda t, n: outs[t, n]),
                                _layernorm(lambda t: _statistics(moments[t]), stream(j), into(lnb, slot)))))

    def b_inputs(j, operand=0):
        def keys(g, t, k):
            kf[j & 1, t, g] = _cat([k, jnp.zeros((16, T), F32)]).astype(BF16).T

        def values(g, t, v):
            for u in range(2):
                i, b, h = 2 * j + t, 56 * u, 4 * g + 2 * u
                vext[i, h] = _cat([v[b:b + 24], jnp.where(low, v[b + 24:b + 32], 1.0)]).astype(BF16)
                vext[i, h + 1] = _cat([jnp.where(low, 1.0, v[b + 24:b + 32]), v[b + 32:b + 56]]).astype(BF16)

        def queries(g, t, q):
            qf[j & 1, t, g] = (q * (DH ** -0.5 * LOG2E)).astype(BF16)

        def matmuls():
            for slot, finish in ((BK, keys), (BV, values), (BQ, queries)):
                yield from project(slot, (lnb, operand), finish)

        return dict(F=matmuls())

    def b_attention_tile(j, t):
        i = 2 * j + t
        nb = min(i + 1, 3) if isinstance(i, int) else 3
        r0 = (160, 32, 0)[nb - 1]
        quarter = lane >> 5
        above = [sub + 8 * n > (lane & 31) for n in range(4)]
        zero = jnp.zeros((8, T), U32)
        tops, probs = [], [[None] * 20 for _ in range(H)]

        def skew_keys(g):
            odd = ((lane >= 28) & (lane < 56)) | (lane >= 84)
            upper = lane >= 56
            kt = _slabs(_load(kf, j & 1, t, g))
            rows = ([zero] * 6 if nb == 1 else _slabs(kprev[g])) + kt
            kprev[g] = _cat(kt[2:])
            lvl = [[jnp.where(odd, rows[n + 2 * (1 - b)], rows[n + 2 * b]) for n in range(12)] for b in range(2)]
            for m in range(4):
                a, b = lvl[m & 1], m >> 1
                kx[i, g, m] = _cat([jnp.where(upper, a[n + 4 * (1 - b)], a[n + 4 * b]) for n in range(8)])

        def score(g, m):
            qm = []
            for n, q in enumerate(_slabs(_load(qf, j & 1, t, g))):
                h0, h1 = 16 * n // DH, (16 * n + 15) // DH
                head = h0 if h0 == h1 else jnp.where(sub < (DH * h1 - 16 * n) // 2, h0, h1)
                qm.append(jnp.where(quarter == (head ^ m), q, zero))
            qm = _bf16(_cat(qm + [zero]))
            keys = [kx[i - 2, g, m, 48:64, :]] if nb == 3 else []
            keys += [kx[i - n, g, m] for n in reversed(range(min(nb, 2)))]
            keys = _cat(keys)
            half = keys.shape[0] // 2
            return _cat([_dot(_bf16(keys[:half]), qm), _dot(_bf16(keys[half:]), qm)])

        def mask(s):
            if nb == 3:
                return [jnp.where(above[n], s[n], s[32 + n]) for n in range(4)] + s[4:32]
            s = s[:-4] + [jnp.where(above[n], NEG, s[n - 4]) for n in range(4)]
            return [jnp.where(quarter >= 3 - n // 4, v, NEG) if n < 12 else v for n, v in enumerate(s)]

        def skews():
            for g in range(NG):
                skew_keys(g)
                yield

        def scores():
            for n in range(H):
                s = mask(_slabs(score(n // 4, n % 4)))
                sbuf[t, n, 0:8 * len(s), :] = _cat(s)
                tops.append(_tree([functools.reduce(jnp.maximum, s[c::2]) for c in range(2)], jnp.maximum))
                if n % 2:
                    yield

        def shifted(mask, moved, kept, n, by):
            a = moved[n - by] if n >= by else None
            b = kept[n] if n < len(kept) else None
            if a is None and b is None:
                return None
            return jnp.where(mask, zero if a is None else a, zero if b is None else b)

        def softmaxes():
            first, blocks = r0 // 32, min(36 - r0 // 8, 32) // 4
            for n in range(0, H, 2):
                top = [_allreduce([tops[n + u]], jnp.maximum, (4, 2, 1)) for u in range(2)]
                ps = [[None] * 18, [None] * 18]
                for b in range(blocks):
                    for u in range(2):
                        e = [jnp.exp2(v - top[u]) for v in _slabs(sbuf[t + z, n + u, 32 * b:32 * b + 32, :])]
                        parts = {first + b: e}
                        if nb == 3 and b == 0:
                            parts = {0: [jnp.where(above[c], e[c], 0.0) for c in range(4)],
                                     8: [jnp.where(above[c], 0.0, e[c]) for c in range(4)]}
                        for at, v in parts.items():
                            pst[u] = _cat(v).astype(BF16)
                            ps[u][2 * at:2 * at + 2] = _slabs(_load(pst, u))
                    for row in range(2 * (first + b), 2 * (first + b) + 2 if b + 1 < blocks else 20):
                        for u in range(2):
                            probs[n + u][row] = shifted((quarter & 1) == 1, ps[1 - u], ps[u], row, 2)
                    if (b + 1) % (blocks // 4) == 0:
                        yield

        def normalize(oa, ob):
            rc = _recip(jnp.where(low, ob[0:8], oa[24:32]))
            sw = pltpu.roll(rc, 4, 0)
            ra, rb = jnp.where(low, sw, rc), jnp.where(low, rc, sw)
            return ([oa[8 * n:8 * n + 8] * ra for n in range(3)]
                    + [jnp.where(low, oa[24:32], ob[0:8]) * sw]
                    + [ob[8 * n:8 * n + 8] * rb for n in range(1, 4)])

        def values():
            for g in range(NG):
                ps, res = probs[4 * g:4 * g + 4], {}
                for h in (0, 2, 1, 3):
                    ph = [shifted(quarter >= 2, ps[h ^ 2], ps[h], row, 4) for row in range(8 * (3 - nb), 24)]
                    vt = _bf16(_cat([_load(vext, i - (nb - 1) + n, 4 * g + h) for n in range(nb)], axis=1))
                    res[h] = _dot(vt, _bf16(_cat(ph)))
                o = normalize(res[0], res[1]) + normalize(res[2], res[3])
                att[j & 1, t, 112 * g:112 * g + 112, :] = _cat(o)
                yield

        return dict(x=skews(), S=scores(), s=softmaxes(), P=values())

    def b_attention(j):
        tiles = [b_attention_tile(j, t) for t in range(2)]

        def both(name):
            for tile in tiles:
                yield from tile[name]

        return {name: both(name) for name in tiles[0]}

    def b_output(j, last):
        def finish(g, t, y):
            rows = pl.ds(112 * g, 112)
            ost[j, rows, T * t:T * t + T] = (xs[2 * j + t, rows, :] + y).astype(BF16)

        moments = ([], [])
        stages = dict(c=_operands(into(lat, 0), lambda t, n: att[j & 1, t, 8 * n:8 * n + 8, :]),
                      O=project(BO, (lat, 0), finish if last else residual(j, moments)))
        if not last:
            stages["o"] = _layernorm(lambda t: _statistics(moments[t]), stream(j), into(lna, j))
        return stages

    def run(order, *stages):
        gens = {name: gen for stage in stages if stage for name, gen in stage.items()}
        for name in order:
            if name in gens:
                next(gens[name])
        for name, gen in gens.items():
            finished = next(gen, "done")
            assert finished == "done", name

    def loop(lo, hi, body):
        lax.fori_loop(lo, hi, lambda j, carry: body(j), None)

    def static(i, value):
        return isinstance(i, int) and i == value

    def input_tile(i, rows):
        return xin[rows, cols(i, T)].astype(F32)

    def input_statistics(j):
        for t in range(2):
            moments = []
            for g in range(NG):
                moments.append(_moments(input_tile(2 * j + t, pl.ds(112 * g, 112))))
                if g == NG - 1:
                    stats[2 * j + t] = _cat(_statistics(moments))
                if g % 2:
                    yield

    def norm_input(j):
        def load(t, n):
            x = input_tile(2 * j + t, pl.ds(8 * n, 8))
            xs[2 * j + t, 8 * n:8 * n + 8, :] = x
            return x

        return _layernorm(lambda t: _slabs(stats[2 * j + t]), load, into(lna, j))

    def pass0(j):
        run(ORDER0, a_keys(j), a_queries(j - 1), dict(n=norm_input(j + 1), m=input_statistics(jnp.minimum(j + 2, NPAIR - 1))))

    def arrive(*pending):
        for cp in pending:
            cp.wait()
        yield from ()

    def chain(*gens):
        for gen in gens:
            yield from gen

    def bridge(order, *stages):
        run(order, *stages, a_keys(NPAIR - 1), dict(z=a_finalize()), a_output(0, "Aba", 1), b_inputs(0, 1),
            a_output(1, "Ede"), a_queries(NPAIR - 1), a_queries(NPAIR - 2, "Rt", 2))

    copies[1].wait()
    copies[2].wait()
    run("wwwwnnnnwwnnnn", dict(n=chain(input_statistics(0), norm_input(0))), dict(
        w=chain(transpose_weight(wa_in, 384, 896),
                weight_operands(AK, 1, bd))))
    run(START, a_keys(0, True), dict(n=chain(input_statistics(1), norm_input(1)), m=input_statistics(2)), dict(
        w=chain(arrive(copies[3]), transpose_weight(wa_in, 896, 3 * D), weight_operands(AV, 2),
                arrive(copies[4], copies[5]), transpose_weight(wa_in, 0, 384), weight_operands(AQ, 0, bd))))
    copies[6].wait()
    for cp in copies[7:]:
        cp.start()
    loop(1, NPAIR - 1, pass0)
    bridge(BRIDGE0, dict(
        w=chain(arrive(*copies[7:]), transpose_weight(woa_in, 0, D), weight_operands(AO, 0),
                transpose_weight(wb_in, 0, 3 * D), weight_operands(BK, 1),
                weight_operands(BV, 2), weight_operands(BQ, 0), transpose_weight(wob_in, 0, D), weight_operands(BO, 0))))

    def pass1(j):
        more, later = not static(j, NPAIR - 1), not static(j, 0)
        run(ORDER1 if more and later else FIRST if more else LAST1, b_attention(j),
            more and later and a_output(j + 1), more and b_inputs(j + 1), later and b_output(j - 1, False),
            later and a_keys(j - 1), more and later and a_queries(j - 1))

    kv[...] = jnp.zeros(kv.shape, F32)
    pass1(0)
    loop(1, NPAIR - 1, pass1)
    pass1(NPAIR - 1)
    bridge(BRIDGE1, b_output(NPAIR - 1, False))

    def pass2(j):
        more, later = not static(j, NPAIR - 1), not static(j, 0)
        run(ORDER2 if more and later else FIRST if more else LAST2, b_attention(j),
            more and later and a_output(j + 1), more and b_inputs(j + 1), later and b_output(j - 1, True))
        if later:
            out_copy(j - 1).start()

    pass2(0)
    loop(1, NPAIR - 1, pass2)
    pass2(NPAIR - 1)
    run("ccccOOOOOOO", b_output(NPAIR - 1, True))
    out_copy(NPAIR - 1).start()
    for j in range(NPAIR):
        out_copy(j).wait()


@jax.jit
def pallas_interleave_layers__linear_kernel_hedgehog__sliding_block__prompt_kernel(
        A_x, A_wqkv, A_w_phi, A_wo, B_x, B_wqkv, B_wo):
    del B_x
    xt = A_x.reshape(S, D).T
    wphi = A_w_phi.transpose(1, 0, 2).reshape(DH * H, DH)
    vmem = pltpu.VMEM
    out = pl.pallas_call(
        _kernel,
        out_shape=jax.ShapeDtypeStruct((D, S), BF16),
        in_specs=[pl.BlockSpec(memory_space=pl.ANY)] * 6,
        out_specs=pl.BlockSpec(memory_space=pl.ANY),
        scratch_shapes=[
            vmem((D, S), BF16), vmem((D, 3 * D), BF16), vmem((DH * H, DH), BF16), vmem((D, D), BF16),
            vmem((D, 3 * D), BF16), vmem((D, D), BF16), vmem((NPAIR, D, 2 * T), BF16),
            vmem((4, 3 * D, 128), F32), vmem((8, 7, 2, 2, 112, 128), BF16),
            vmem((NTILE, D, T), F32), vmem((NPAIR, 7, HALF, T), BF16), vmem((NTILE, NP, 112, T), BF16),
            vmem((NP, 64, 112), F32), vmem((NP, 64, 112), BF16), vmem((2, 7, HALF, T), BF16),
            vmem((2, 2, D, T), F32), vmem((2, 2, NG, 112, T), BF16), vmem((2, 2, NG, T, 128), BF16),
            vmem((NG, 48, 128), U32), vmem((NTILE, NG, 4, T // 2, 128), U32), vmem((NTILE, H, 32, T), BF16),
            vmem((3, 2, D, T), F32), vmem((NP, 2, 112, T), BF16),
            vmem((1, 7, HALF, T), BF16), vmem((1, 7, HALF, T), BF16),
            vmem((2, H, 256, T), F32), vmem((NTILE, 16, T), F32), vmem((2, 32, T), BF16),
            pltpu.SMEM((1,), jnp.int32), pltpu.SemaphoreType.DMA((10,)),
            pltpu.SemaphoreType.DMA((NPAIR,)),
        ],
        compiler_params=pltpu.CompilerParams(vmem_limit_bytes=64 << 20),
    )(xt, A_wqkv, wphi, A_wo, B_wqkv, B_wo)
    return out.T.reshape(1, S, D)
```
